```python
import os as _os
_os.environ.setdefault("JAX_PLATFORMS", "cpu")
import jax
import jax.numpy as jnp

def _softmax(x, axis=-1):
    return jax.nn.softmax(x, axis=axis)
def _gelu(x):
    return jax.nn.gelu(x, approximate=True)
def _silu(x):
    return jax.nn.silu(x)
def _sigmoid(x):
    return jax.nn.sigmoid(x)
def _layernorm(x, axis=-1, eps=1e-5):
    m = jnp.mean(x, axis=axis, keepdims=True)
    v = jnp.var(x, axis=axis, keepdims=True)
    return (x - m) / jnp.sqrt(v + eps)
def _scatter_add(tgt, idx, src, axis=0):
    return tgt.at[idx].add(src)
def _segment_sum(src, seg, n):
    return jax.ops.segment_sum(src, seg, n)
class _Rng:
    def __init__(self, key):
        self._k = key
    def _next(self):
        self._k, sub = jax.random.split(self._k)
        return sub
    def normal(self, shape):
        return jax.random.normal(self._next(), shape, dtype=jnp.bfloat16)
    def randint(self, lo, hi, shape):
        return jax.random.randint(self._next(), shape, lo, hi, dtype=jnp.int32)
    def uniform(self, shape, lo=0.0, hi=1.0):
        return jax.random.uniform(self._next(), shape, jnp.bfloat16, lo, hi)
    def permutation(self, n):
        return jax.random.permutation(self._next(), n)


kernel_name = 'gated_mix__mha_block__mha_block__prompt'

def setup_inputs():
    _rng = _Rng(jax.random.key(int.from_bytes(__import__("os").urandom(4), "little")))
    _w = (lambda a: (lambda t: t.astype(jnp.bfloat16) if jnp.issubdtype(t.dtype, jnp.floating) else t)(jnp.asarray(a)))
    def _A_setup():
        B, S, D, H = 1, 2048, 448, 16
        return {
            "x": _w((lambda *s: _rng.normal(s) * 0.05)(B, S, D)),
            "wqkv": _w((lambda *s: _rng.normal(s) * 0.4)(D, 3 * D)),
            "wo": _w((lambda *s: _rng.normal(s) * 0.05)(D, D)),
        }
    _A_in = _A_setup()

    def _B_setup():
        B, S, D, H = 1, 2048, 448, 16
        return {
            "x": _w((lambda *s: _rng.normal(s) * 0.05)(B, S, D)),
            "wqkv": _w((lambda *s: _rng.normal(s) * 0.4)(D, 3 * D)),
            "wo": _w((lambda *s: _rng.normal(s) * 0.05)(D, D)),
        }
    _B_in = _B_setup()

    return {
        "A_x": _A_in["x"],
        "A_wqkv": _A_in["wqkv"],
        "A_wo": _A_in["wo"],
        "B_x": _B_in["x"],
        "B_wqkv": _B_in["wqkv"],
        "B_wo": _B_in["wo"],
        "gate_w": _w((lambda *s: _rng.normal(s) * 0.05)(448) * 16.0),
    }

def reference(A_x, A_wqkv, A_wo, B_x, B_wqkv, B_wo, gate_w):
    def _A_ref(x, wqkv, wo):
        B, S, D = x.shape
        H = 16
        Dh = D // H
        qkv = (lambda x, *d: x.transpose(*d))((x @ wqkv).reshape(B, S, 3, H, Dh), 2, 0, 3, 1, 4)
        q, k, v = qkv[0], qkv[1], qkv[2]
        scores = jnp.einsum("bhqd,bhkd->bhqk", q, k) * (Dh ** -0.5)
        p = _softmax(scores, axis=-1)
        o = jnp.einsum("bhqk,bhkd->bhqd", p, v)
        return (lambda x, *d: x.transpose(*d))(o, 0, 2, 1, 3).reshape(B, S, D) @ wo

    def _B_ref(x, wqkv, wo):
        B, S, D = x.shape
        H = 16
        Dh = D // H
        qkv = (lambda x, *d: x.transpose(*d))((x @ wqkv).reshape(B, S, 3, H, Dh), 2, 0, 3, 1, 4)
        q, k, v = qkv[0], qkv[1], qkv[2]
        scores = jnp.einsum("bhqd,bhkd->bhqk", q, k) * (Dh ** -0.5)
        p = _softmax(scores, axis=-1)
        o = jnp.einsum("bhqk,bhkd->bhqd", p, v)
        return (lambda x, *d: x.transpose(*d))(o, 0, 2, 1, 3).reshape(B, S, D) @ wo

    x = A_x
    g = _sigmoid((x * gate_w).sum(-1, keepdims=True))
    a = _A_ref(x, A_wqkv, A_wo)
    b = _B_ref(x, B_wqkv, B_wo)
    return g * a + (1 - g) * b
```

```python
import math
import jax
import jax.numpy as jnp
import jax.experimental.pallas as pl
import jax.experimental.pallas.tpu as pltpu

S, D, H, DH, DP = 2048, 448, 16, 28, 32
HP = H * DP
DK = 512
TQ = 512
KC = 128
NQ = S // TQ
NIT = 2 * H * NQ
NC = S // KC
PC = 512
UN = 8
OC = 512

def _kernel(xT_hbm, wA_hbm, woA_hbm, wB_hbm, woB_hbm, gw_ref, o_hbm,
            xT_ref, w_ref, wo_ref, o_buf, sems,
            x_scr, wpad_scr, wpadb_scr, wopad_scr, woT_scr, g_scr, qT_scr, k_scr, vT_scr, oT_scr, sA, sB, mA, mB):
    f32, bf16 = jnp.float32, jnp.bfloat16
    cps = [pltpu.make_async_copy(src, dst, sems.at[i]) for i, (src, dst) in enumerate(
        ((xT_hbm, xT_ref.at[0:D, :]), (wA_hbm, w_ref.at[0]), (wB_hbm, w_ref.at[1]),
         (woA_hbm, wo_ref.at[0]), (woB_hbm, wo_ref.at[1])))]
    for cp in cps:
        cp.start()
    scale = (DH ** -0.5) * math.log2(math.e)
    r64 = jax.lax.broadcasted_iota(jnp.int32, (DK - D, S), 0)
    xT_ref[D:DK, :] = jnp.where(r64 == 0, 1.0, 0.0).astype(bf16)
    rr = jax.lax.broadcasted_iota(jnp.int32, (3 * HP, DK), 0)
    cc = jax.lax.broadcasted_iota(jnp.int32, (3 * HP, DK), 1)
    wpad_scr[...] = jnp.where((rr >= 2 * HP) & (rr % DP == DH) & (cc == D), 1.0, 0.0)
    wopad_scr[...] = jnp.zeros_like(wopad_scr)
    cps[0].wait()
    x_scr[...] = xT_ref[...].T
    nt = (((1,), (1,)), ((), ()))

    gl = jnp.dot(jnp.broadcast_to(gw_ref[...], (8, D)), xT_ref[0:D, :], preferred_element_type=f32)[0:1, :]
    gate = jax.nn.sigmoid(gl)
    g_scr[0:1, :] = gate
    g_scr[1:2, :] = 1.0 - gate
    cps[1].wait()
    cps[2].wait()

    def blk_body(blk, carry):
        wT = w_ref[blk].T.astype(f32)
        for i in range(3 * H):
            wpad_scr[i * DP:i * DP + DH, 0:D] = wT[i * DH:(i + 1) * DH, :]
        wpadb_scr[...] = wpad_scr[...].astype(bf16)
        b0 = pl.multiple_of(blk * HP, HP)

        def proj(c, carry):
            c0 = pl.multiple_of(c * PC, PC)
            xTc = xT_ref[:, pl.ds(c0, PC)]
            k_scr[pl.ds(c0, PC), pl.ds(b0, HP)] = jax.lax.dot_general(
                x_scr[pl.ds(c0, PC), :], wpadb_scr[HP:2 * HP, :], nt, preferred_element_type=f32).astype(bf16)
            qT = jnp.dot(wpadb_scr[0:HP, :], xTc, preferred_element_type=f32)
            qT_scr[pl.ds(b0, HP), pl.ds(c0, PC)] = (qT * scale).astype(bf16)
            vT_scr[pl.ds(b0, HP), pl.ds(c0, PC)] = jnp.dot(wpadb_scr[2 * HP:3 * HP, :], xTc, preferred_element_type=f32).astype(bf16)
            return carry
        jax.lax.fori_loop(0, S // PC, proj, 0)
        return carry
    jax.lax.fori_loop(0, 2, blk_body, 0)

    def step(it_qk, s_nxt, m_nxt, it_pv, s_cur, m_cur):
        if it_qk is not None:
            h = it_qk // NQ
            qb = it_qk % NQ
            g = h // 4
            j = h % 4
            g0 = pl.multiple_of(g * 128, 128)
            q0 = pl.multiple_of(qb * TQ, TQ)
            qg = qT_scr[pl.ds(g0, 128), pl.ds(q0, TQ)]
            rid = jax.lax.broadcasted_iota(jnp.int32, (128, 1), 0) // DP
            qm = jnp.where(rid == j, qg, jnp.zeros_like(qg))
        if it_pv is not None:
            h2 = it_pv // NQ
            qb2 = it_pv % NQ
            q02 = pl.multiple_of(qb2 * TQ, TQ)
            h02 = pl.multiple_of(h2 * DP, DP)
            mc = m_cur[...]
        mx = None
        o = None
        for c in range(NC):
            if it_qk is not None:
                kg = k_scr[c * KC:(c + 1) * KC, pl.ds(g0, 128)]
                s = jnp.dot(kg, qm, preferred_element_type=f32)
                s_nxt[c * KC:(c + 1) * KC, :] = s
                sm = jnp.max(s.reshape(KC // 8, 8, TQ), axis=0)
                mx = sm if mx is None else jnp.maximum(mx, sm)
            if it_pv is not None:
                p = jnp.exp2(s_cur[c * KC:(c + 1) * KC, :] - mc).astype(bf16)
                vt = vT_scr[pl.ds(h02, DP), c * KC:(c + 1) * KC]
                oc = jnp.dot(vt, p, preferred_element_type=f32)
                o = oc if o is None else o + oc
        if it_qk is not None:
            m_nxt[...] = jnp.max(mx, axis=0, keepdims=True)
        if it_pv is not None:
            r = g_scr[pl.ds(h2 // H, 1), pl.ds(q02, TQ)] / o[DH:DH + 1, :]
            oT_scr[pl.ds(h02, DP), pl.ds(q02, TQ)] = (o * r).astype(bf16)

    step(0, sA, mA, None, None, None)
    def body(i, c):
        for u in range(UN // 2):
            it = UN * i + 2 * u
            step(it + 1, sB, mB, it, sA, mA)
            step(it + 2, sA, mA, it + 1, sB, mB)
        return c
    jax.lax.fori_loop(0, NIT // UN - 1, body, 0)
    for u in range(UN // 2):
        it = NIT - UN + 2 * u
        step(it + 1, sB, mB, it, sA, mA)
        step(it + 2 if it + 2 < NIT else None, sA, mA, it + 1, sB, mB)

    cps[3].wait()
    cps[4].wait()
    for blk in range(2):
        wo = wo_ref[blk].astype(f32)
        for i in range(H):
            wopad_scr[blk * HP + i * DP:blk * HP + i * DP + DH, :] = wo[i * DH:(i + 1) * DH, :]
    woT_scr[...] = wopad_scr[...].astype(bf16).T

    def ocopy(c):
        c0 = pl.multiple_of(c * OC, OC)
        return pltpu.make_async_copy(o_buf.at[:, pl.ds(c0, OC)], o_hbm.at[:, pl.ds(c0, OC)], sems.at[5 + c])
    def oproj(c, carry):
        c0 = pl.multiple_of(c * OC, OC)
        o_buf[:, pl.ds(c0, OC)] = jnp.dot(woT_scr[...], oT_scr[:, pl.ds(c0, OC)], preferred_element_type=f32).astype(bf16)
        ocopy(c).start()
        return carry
    jax.lax.fori_loop(0, S // OC, oproj, 0)
    for c in range(S // OC):
        ocopy(c).wait()


@jax.jit
def pallas_gated_mix__mha_block__mha_block__prompt_kernel(A_x, A_wqkv, A_wo, B_x, B_wqkv, B_wo, gate_w):
    xT = A_x.reshape(S, D).T
    any_spec = pl.BlockSpec(memory_space=pl.ANY)
    outT = pl.pallas_call(
        _kernel,
        out_shape=jax.ShapeDtypeStruct((D, S), jnp.bfloat16),
        in_specs=[any_spec] * 5 + [pl.BlockSpec(memory_space=pltpu.VMEM)],
        out_specs=any_spec,
        scratch_shapes=[
            pltpu.VMEM((DK, S), jnp.bfloat16),
            pltpu.VMEM((2, D, 3 * D), jnp.bfloat16),
            pltpu.VMEM((2, D, D), jnp.bfloat16),
            pltpu.VMEM((D, S), jnp.bfloat16),
            pltpu.SemaphoreType.DMA((5 + S // OC,)),
            pltpu.VMEM((S, DK), jnp.bfloat16),
            pltpu.VMEM((3 * HP, DK), jnp.float32),
            pltpu.VMEM((3 * HP, DK), jnp.bfloat16),
            pltpu.VMEM((2 * HP, D), jnp.float32),
            pltpu.VMEM((D, 2 * HP), jnp.bfloat16),
            pltpu.VMEM((8, S), jnp.float32),
            pltpu.VMEM((2 * HP, S), jnp.bfloat16),
            pltpu.VMEM((S, 2 * HP), jnp.bfloat16),
            pltpu.VMEM((2 * HP, S), jnp.bfloat16),
            pltpu.VMEM((2 * HP, S), jnp.bfloat16),
            pltpu.VMEM((S, TQ), jnp.float32),
            pltpu.VMEM((S, TQ), jnp.float32),
            pltpu.VMEM((1, TQ), jnp.float32),
            pltpu.VMEM((1, TQ), jnp.float32),
        ],
        compiler_params=pltpu.CompilerParams(vmem_limit_bytes=100 * 1024 * 1024),
    )(xT, A_wqkv, A_wo, B_wqkv, B_wo, gate_w.reshape(1, D))
    return outT.T.reshape(1, S, D)
```

```python
import math
import jax
import jax.numpy as jnp
import jax.experimental.pallas as pl
import jax.experimental.pallas.tpu as pltpu

S, D, H, DH, DP = 2048, 448, 16, 28, 32
HP = H * DP
GW = 4 * DH
TQ = 1024
KC = 128
NQ = S // TQ
NIT = 2 * H * NQ
NC = S // KC
PC = 512
NP = S // PC
UN = 4
SUB = 512
OC = 512
NO = S // OC

def _kernel(xT_hbm, wA_hbm, woA_hbm, wB_hbm, woB_hbm, gw_ref, o_hbm,
            xT_ref, w_ref, wo_ref, o_buf, sems,
            wqv_scr, wk_scr, wopad_scr, woT_scr, g_scr, qT_scr, k_scr, vT_scr, oT_scr, sA, sB, mA, mB):
    f32, bf16 = jnp.float32, jnp.bfloat16
    def xcopy(c):
        c0 = pl.multiple_of(c * PC, PC)
        return pltpu.make_async_copy(xT_hbm.at[:, pl.ds(c0, PC)], xT_ref.at[:, pl.ds(c0, PC)], sems.at[4 + c])
    cps = [pltpu.make_async_copy(src, dst, sems.at[i]) for i, (src, dst) in enumerate(
        ((wA_hbm, w_ref.at[0]), (wB_hbm, w_ref.at[1]), (woA_hbm, wo_ref.at[0]), (woB_hbm, wo_ref.at[1])))]
    cps[0].start()
    for c in range(NP):
        xcopy(c).start()
    for cp in cps[1:]:
        cp.start()
    scale = (DH ** -0.5) * math.log2(math.e)
    r16 = jax.lax.broadcasted_iota(jnp.int32, (16, S), 0)
    slab = jnp.where(r16 == DH - 16, 1.0, 0.0).astype(bf16)
    for i in range(2 * H):
        vT_scr[i * DP + 16:(i + 1) * DP, :] = slab
    wk_scr[...] = jnp.zeros_like(wk_scr)
    wopad_scr[...] = jnp.zeros_like(wopad_scr)
    qT_scr[2 * D:2 * D + 16, :] = jnp.zeros((16, S), bf16)
    nt = (((1,), (1,)), ((), ()))
    gw8 = jnp.broadcast_to(gw_ref[...], (8, D))

    def step(it_qk, s_nxt, m_nxt, it_pv, s_cur, m_cur, extra=None):
        if it_qk is not None:
            h = it_qk // NQ
            qb = it_qk % NQ
            g = h // 4
            j = h % 4
            g0 = pl.multiple_of(g * 128, 128)
            gq0 = pl.multiple_of(g * GW, 16)
            q0 = pl.multiple_of(qb * TQ, TQ)
            qg = qT_scr[pl.ds(gq0, 128), pl.ds(q0, TQ)]
            rid = jax.lax.broadcasted_iota(jnp.int32, (128, 1), 0) - j * DH
            qm = jnp.where((rid >= 0) & (rid < DH), qg, jnp.zeros_like(qg))
        if it_pv is not None:
            h2 = it_pv // NQ
            qb2 = it_pv % NQ
            q02 = pl.multiple_of(qb2 * TQ, TQ)
            h02 = pl.multiple_of(h2 * DP, DP)
            mc = m_cur[...]
        NS = TQ // SUB
        mx = [None] * NS
        o = [None] * NS
        for c in range(NC):
            if it_qk is not None:
                kg = k_scr[c * KC:(c + 1) * KC, pl.ds(g0, 128)]
            if it_pv is not None:
                vt = vT_scr[pl.ds(h02, DP), c * KC:(c + 1) * KC]
            for u in range(NS):
                cs = slice(u * SUB, (u + 1) * SUB)
                if it_qk is not None:
                    s = jnp.dot(kg, qm[:, cs], preferred_element_type=f32)
                    s_nxt[c * KC:(c + 1) * KC, cs] = s
                    sm = jnp.max(s.reshape(KC // 8, 8, SUB), axis=0)
                    mx[u] = sm if mx[u] is None else jnp.maximum(mx[u], sm)
                if extra is not None and u == 0:
                    extra(c)
                if it_pv is not None:
                    p = jnp.exp2(s_cur[c * KC:(c + 1) * KC, cs] - mc[:, cs]).astype(bf16)
                    oc = jnp.dot(vt, p, preferred_element_type=f32)
                    o[u] = oc if o[u] is None else o[u] + oc
        for u in range(NS):
            cs = slice(u * SUB, (u + 1) * SUB)
            if it_qk is not None:
                m_nxt[:, cs] = jnp.max(mx[u], axis=0, keepdims=True)
            if it_pv is not None:
                qq = pl.multiple_of(q02 + u * SUB, SUB)
                r = g_scr[pl.ds(h2 // H, 1), pl.ds(qq, SUB)] / o[u][DH:DH + 1, :]
                oT_scr[pl.ds(h02, DP), pl.ds(qq, SUB)] = (o[u] * r).astype(bf16)

    def wo_prep(c):
        if c < 2:
            wo = wo_ref[c].astype(f32)
            for i in range(H):
                wopad_scr[c * HP + i * DP:c * HP + i * DP + DH, :] = wo[i * DH:(i + 1) * DH, :]
        elif c < 10:
            k0 = (c - 2) * 128
            woT_scr[:, k0:k0 + 128] = wopad_scr[k0:k0 + 128, :].astype(bf16).T

    def ocopy(c):
        c0 = pl.multiple_of(c * OC, OC)
        return pltpu.make_async_copy(o_buf.at[:, pl.ds(c0, OC)], o_hbm.at[:, pl.ds(c0, OC)], sems.at[4 + NP + c])

    def oproj_early(c):
        nt_ = (S - TQ) // 128
        per = -(-nt_ // NC)
        for t in range(c * per, min((c + 1) * per, nt_)):
            n0 = t * 128
            o_buf[:, n0:n0 + 128] = jnp.dot(woT_scr[...], oT_scr[:, n0:n0 + 128], preferred_element_type=f32).astype(bf16)

    def wprep(blk, part):
        lo, hi = part
        wT = w_ref[blk, :, lo:hi].T
        def put(dst, d0, r0, r1):
            a, b = max(r0, lo), min(r1, hi)
            if a < b:
                dst[d0 + a - r0:d0 + b - r0, :] = wT[a - lo:b - lo, :]
        put(wqv_scr, 0, 0, D)
        put(wqv_scr, D, 2 * D, 3 * D)
        for g in range(4):
            put(wk_scr, g * 128, D + g * GW, D + (g + 1) * GW)
    wparts = [(0, 384), (384, 768), (768, 1152), (1152, 1344)]

    def extra0(c):
        wo_prep(c)
        if 10 <= c < 10 + len(wparts):
            wprep(1, wparts[c - 10])

    def blk_body(blk, carry):
        b0 = pl.multiple_of(blk * HP, HP)
        bq0 = pl.multiple_of(blk * D, 16)

        def proj(c, carry):
            @pl.when(blk == 0)
            def _():
                xcopy(c).wait()
            c0 = pl.multiple_of(c * PC, PC)
            xTd = xT_ref[:, pl.ds(c0, PC)]
            qT = jnp.dot(wqv_scr[0:D, :], xTd, preferred_element_type=f32)
            qT_scr[pl.ds(bq0, D), pl.ds(c0, PC)] = (qT * scale).astype(bf16)
            vT = jnp.dot(wqv_scr[D:2 * D, :], xTd, preferred_element_type=f32)
            for i in range(H):
                vT_scr[pl.ds(pl.multiple_of(b0 + i * DP, DP), DH), pl.ds(c0, PC)] = vT[i * DH:(i + 1) * DH, :].astype(bf16)
            k_scr[pl.ds(c0, PC), pl.ds(b0, HP)] = jax.lax.dot_general(
                xTd.T, wk_scr[...], nt, preferred_element_type=f32).astype(bf16)
            gate = jax.nn.sigmoid(jnp.dot(gw8, xTd, preferred_element_type=f32)[0:1, :])
            g_scr[0:1, pl.ds(c0, PC)] = gate
            g_scr[1:2, pl.ds(c0, PC)] = 1.0 - gate
            return carry
        jax.lax.fori_loop(0, NP, proj, 0)

        @pl.when(blk == 0)
        def _():
            for cp in cps[1:]:
                cp.wait()
            step(0, sA, mA, None, None, None, extra=extra0)
        return carry

    cps[0].wait()
    for part in wparts:
        wprep(0, part)
    jax.lax.fori_loop(0, 2, blk_body, 0)

    def body(i, c):
        for u in range(UN // 2):
            it = UN * i + 2 * u
            step(it + 1, sB, mB, it, sA, mA)
            step(it + 2, sA, mA, it + 1, sB, mB)
        return c
    jax.lax.fori_loop(0, NIT // UN - 1, body, 0)
    for u in range(UN // 2):
        it = NIT - UN + 2 * u
        step(it + 1, sB, mB, it, sA, mA)
        if it + 2 < NIT:
            step(it + 2, sA, mA, it + 1, sB, mB)
        else:
            step(None, sA, mA, it + 1, sB, mB, extra=oproj_early)
    ne = (S - TQ) // OC
    for c in range(ne):
        ocopy(c).start()
    def oproj(c, carry):
        c0 = pl.multiple_of(c * OC, OC)
        o_buf[:, pl.ds(c0, OC)] = jnp.dot(woT_scr[...], oT_scr[:, pl.ds(c0, OC)], preferred_element_type=f32).astype(bf16)
        ocopy(c).start()
        return carry
    jax.lax.fori_loop(ne, NO, oproj, 0)
    for c in range(NO):
        ocopy(c).wait()


@jax.jit
def pallas_gated_mix__mha_block__mha_block__prompt_kernel(A_x, A_wqkv, A_wo, B_x, B_wqkv, B_wo, gate_w):
    xT = A_x.reshape(S, D).T
    any_spec = pl.BlockSpec(memory_space=pl.ANY)
    outT = pl.pallas_call(
        _kernel,
        out_shape=jax.ShapeDtypeStruct((D, S), jnp.bfloat16),
        in_specs=[any_spec] * 5 + [pl.BlockSpec(memory_space=pltpu.VMEM)],
        out_specs=any_spec,
        scratch_shapes=[
            pltpu.VMEM((D, S), jnp.bfloat16),
            pltpu.VMEM((2, D, 3 * D), jnp.bfloat16),
            pltpu.VMEM((2, D, D), jnp.bfloat16),
            pltpu.VMEM((D, S), jnp.bfloat16),
            pltpu.SemaphoreType.DMA((4 + NP + NO,)),
            pltpu.VMEM((2 * D, D), jnp.bfloat16),
            pltpu.VMEM((HP, D), jnp.bfloat16),
            pltpu.VMEM((2 * HP, D), jnp.float32),
            pltpu.VMEM((D, 2 * HP), jnp.bfloat16),
            pltpu.VMEM((8, S), jnp.float32),
            pltpu.VMEM((2 * D + 16, S), jnp.bfloat16),
            pltpu.VMEM((S, 2 * HP), jnp.bfloat16),
            pltpu.VMEM((2 * HP, S), jnp.bfloat16),
            pltpu.VMEM((2 * HP, S), jnp.bfloat16),
            pltpu.VMEM((S, TQ), jnp.float32),
            pltpu.VMEM((S, TQ), jnp.float32),
            pltpu.VMEM((1, TQ), jnp.float32),
            pltpu.VMEM((1, TQ), jnp.float32),
        ],
        compiler_params=pltpu.CompilerParams(vmem_limit_bytes=100 * 1024 * 1024),
    )(xT, A_wqkv, A_wo, B_wqkv, B_wo, gate_w.reshape(1, D))
    return outT.T.reshape(1, S, D)
```

```python
import functools
import math

import jax
import jax.numpy as jnp
import jax.experimental.pallas as pl
import jax.experimental.pallas.tpu as pltpu

S, D, H, DH, DP = 2048, 448, 16, 28, 32
HP = H * DP
GW = 4 * DH
TQ = 1024
KC = 256
SUB = 256
NQ = S // TQ
NIT = 2 * H * NQ
NC = S // KC
NS = TQ // SUB
PC = 512
NP = S // PC
UN = 4
OC = 512
NO = S // OC


def _kernel(xT_hbm, wA_hbm, woA_hbm, wB_hbm, woB_hbm, gw_ref, o_hbm,
            xT_ref, w_ref, wo_ref, o_buf, sems,
            wT_scr, wopad_scr, woT_scr, g_scr, qT_scr, k_scr, vT_scr, oT_scr, sA, sB, mA, mB):
    f32, bf16 = jnp.float32, jnp.bfloat16

    def xcopy(c):
        c0 = pl.multiple_of(c * PC, PC)
        return pltpu.make_async_copy(xT_hbm.at[:, pl.ds(c0, PC)], xT_ref.at[:, pl.ds(c0, PC)], sems.at[4 + c])

    cps = [pltpu.make_async_copy(src, dst, sems.at[i]) for i, (src, dst) in enumerate(
        ((wA_hbm, w_ref.at[0]), (wB_hbm, w_ref.at[1]), (woA_hbm, wo_ref.at[0]), (woB_hbm, wo_ref.at[1])))]
    cps[0].start()
    for c in range(NP):
        xcopy(c).start()
    for cp in cps[1:]:
        cp.start()

    scale = (DH ** -0.5) * math.log2(math.e)
    r16 = jax.lax.broadcasted_iota(jnp.int32, (16, S), 0)
    slab = jnp.where(r16 == DH - 16, 1.0, 0.0).astype(bf16)
    for i in range(2 * H):
        vT_scr[i * DP + 16:(i + 1) * DP, :] = slab
    for g in range(8):
        k_scr[:, g * 128 + GW:(g + 1) * 128] = jnp.zeros((S, 128 - GW), bf16)
    wopad_scr[...] = jnp.zeros_like(wopad_scr)
    qT_scr[2 * D:2 * D + 16, :] = jnp.zeros((16, S), bf16)
    gw8 = jnp.broadcast_to(gw_ref[...], (8, D))

    def step(it_qk, s_nxt, m_nxt, it_pv, s_cur, m_cur, extra=None):
        if it_qk is not None:
            h = it_qk // NQ
            qb = it_qk % NQ
            g = h // 4
            j = h % 4
            g0 = pl.multiple_of(g * 128, 128)
            gq0 = pl.multiple_of(g * GW, 16)
            q0 = pl.multiple_of(qb * TQ, TQ)
            qg = qT_scr[pl.ds(gq0, 128), pl.ds(q0, TQ)]
            rid = jax.lax.broadcasted_iota(jnp.int32, (128, 1), 0) - j * DH
            qm = jnp.where((rid >= 0) & (rid < DH), qg, jnp.zeros_like(qg))
        if it_pv is not None:
            h2 = it_pv // NQ
            qb2 = it_pv % NQ
            q02 = pl.multiple_of(qb2 * TQ, TQ)
            h02 = pl.multiple_of(h2 * DP, DP)
            mc = m_cur[...]
            gr = g_scr[pl.ds(h2 // H, 1), pl.ds(q02, TQ)]
        mx = [None] * NS
        o = [None] * NS
        for c in range(NC):
            if it_qk is not None:
                kg = k_scr[c * KC:(c + 1) * KC, pl.ds(g0, 128)]
            if it_pv is not None:
                vt = vT_scr[pl.ds(h02, DP), c * KC:(c + 1) * KC]
            for u in range(NS):
                cs = slice(u * SUB, (u + 1) * SUB)
                if it_qk is not None:
                    s = jnp.dot(kg, qm[:, cs], preferred_element_type=f32)
                    s_nxt[c * KC:(c + 1) * KC, cs] = s
                    sm = jnp.max(s.reshape(KC // 8, 8, SUB), axis=0)
                    mx[u] = sm if mx[u] is None else jnp.maximum(mx[u], sm)
                if extra is not None:
                    slot, nslot = c * NS + u, NC * NS
                    for t in range(len(extra)):
                        if (t * nslot) // len(extra) == slot:
                            extra[t]()
                if it_pv is not None:
                    p = jnp.exp2(s_cur[c * KC:(c + 1) * KC, cs] - mc[:, cs]).astype(bf16)
                    oc = jnp.dot(vt, p, preferred_element_type=f32)
                    o[u] = oc if o[u] is None else o[u] + oc
        for u in range(NS):
            cs = slice(u * SUB, (u + 1) * SUB)
            if it_qk is not None:
                m_nxt[:, cs] = jnp.max(mx[u], axis=0, keepdims=True)
            if it_pv is not None:
                qq = pl.multiple_of(q02 + u * SUB, SUB)
                r = gr[:, cs] / o[u][DH:DH + 1, :]
                oT_scr[pl.ds(h02, DP), pl.ds(qq, SUB)] = (o[u] * r).astype(bf16)

    def wo_pad(b):
        wo = wo_ref[b].astype(f32)
        for i in range(H):
            wopad_scr[b * HP + i * DP:b * HP + i * DP + DH, :] = wo[i * DH:(i + 1) * DH, :]

    def wo_xpose(k0):
        woT_scr[:, k0:k0 + 128] = wopad_scr[k0:k0 + 128, :].astype(bf16).T

    def wprep(blk, part):
        lo, hi = part
        wT_scr[lo:hi, :] = w_ref[blk, :, lo:hi].T

    wparts = [(0, 384), (384, 768), (768, 1152), (1152, 1344)]
    extra0 = ([functools.partial(wo_pad, b) for b in range(2)]
              + [functools.partial(wo_xpose, k0) for k0 in range(0, 2 * HP, 128)]
              + [functools.partial(wprep, 1, part) for part in wparts])

    def ocopy(c):
        c0 = pl.multiple_of(c * OC, OC)
        return pltpu.make_async_copy(o_buf.at[:, pl.ds(c0, OC)], o_hbm.at[:, pl.ds(c0, OC)], sems.at[4 + NP + c])

    def oproj_tile(n0):
        o_buf[:, n0:n0 + 128] = jnp.dot(woT_scr[...], oT_scr[:, n0:n0 + 128],
                                        preferred_element_type=f32).astype(bf16)

    oproj_early = [functools.partial(oproj_tile, n0) for n0 in range(0, S - TQ, 128)]

    def blk_body(blk, carry):
        b0 = pl.multiple_of(blk * HP, HP)
        bq0 = pl.multiple_of(blk * D, 16)

        def proj(c, carry):
            @pl.when(blk == 0)
            def _():
                xcopy(c).wait()
            c0 = pl.multiple_of(c * PC, PC)
            xTd = xT_ref[:, pl.ds(c0, PC)]
            qT = jnp.dot(wT_scr[0:D, :], xTd, preferred_element_type=f32)
            qT_scr[pl.ds(bq0, D), pl.ds(c0, PC)] = (qT * scale).astype(bf16)
            kT = jnp.dot(wT_scr[D:2 * D, :], xTd, preferred_element_type=f32).astype(bf16)
            for g in range(4):
                k_scr[pl.ds(c0, PC), pl.ds(pl.multiple_of(b0 + g * 128, 128), GW)] = kT[g * GW:(g + 1) * GW, :].T
            vT = jnp.dot(wT_scr[2 * D:3 * D, :], xTd, preferred_element_type=f32)
            for i in range(H):
                vT_scr[pl.ds(pl.multiple_of(b0 + i * DP, DP), DH), pl.ds(c0, PC)] = (
                    vT[i * DH:(i + 1) * DH, :].astype(bf16))
            gate = jax.nn.sigmoid(jnp.dot(gw8, xTd, preferred_element_type=f32)[0:1, :])
            g_scr[0:1, pl.ds(c0, PC)] = gate
            g_scr[1:2, pl.ds(c0, PC)] = 1.0 - gate
            return carry
        jax.lax.fori_loop(0, NP, proj, 0)

        @pl.when(blk == 0)
        def _():
            for cp in cps[1:]:
                cp.wait()
            step(0, sA, mA, None, None, None, extra=extra0)
        return carry

    cps[0].wait()
    for part in wparts:
        wprep(0, part)
    jax.lax.fori_loop(0, 2, blk_body, 0)

    def body(i, c):
        for u in range(UN // 2):
            it = UN * i + 2 * u
            step(it + 1, sB, mB, it, sA, mA)
            step(it + 2, sA, mA, it + 1, sB, mB)
        return c
    jax.lax.fori_loop(0, NIT // UN - 1, body, 0)
    for u in range(UN // 2):
        it = NIT - UN + 2 * u
        step(it + 1, sB, mB, it, sA, mA)
        if it + 2 < NIT:
            step(it + 2, sA, mA, it + 1, sB, mB)
        else:
            step(None, sA, mA, it + 1, sB, mB, extra=oproj_early)

    ne = (S - TQ) // OC
    for c in range(ne):
        ocopy(c).start()

    def oproj(c, carry):
        c0 = pl.multiple_of(c * OC, OC)
        o_buf[:, pl.ds(c0, OC)] = jnp.dot(woT_scr[...], oT_scr[:, pl.ds(c0, OC)],
                                          preferred_element_type=f32).astype(bf16)
        ocopy(c).start()
        return carry
    jax.lax.fori_loop(ne, NO, oproj, 0)
    for c in range(NO):
        ocopy(c).wait()


@jax.jit
def pallas_gated_mix__mha_block__mha_block__prompt_kernel(
    A_x: jax.Array,
    A_wqkv: jax.Array,
    A_wo: jax.Array,
    B_x: jax.Array,
    B_wqkv: jax.Array,
    B_wo: jax.Array,
    gate_w: jax.Array,
):
    del B_x
    xT = A_x.reshape(S, D).T
    any_spec = pl.BlockSpec(memory_space=pl.ANY)
    outT = pl.pallas_call(
        _kernel,
        out_shape=jax.ShapeDtypeStruct((D, S), jnp.bfloat16),
        in_specs=[any_spec] * 5 + [pl.BlockSpec(memory_space=pltpu.VMEM)],
        out_specs=any_spec,
        scratch_shapes=[
            pltpu.VMEM((D, S), jnp.bfloat16),
            pltpu.VMEM((2, D, 3 * D), jnp.bfloat16),
            pltpu.VMEM((2, D, D), jnp.bfloat16),
            pltpu.VMEM((D, S), jnp.bfloat16),
            pltpu.SemaphoreType.DMA((4 + NP + NO,)),
            pltpu.VMEM((3 * D, D), jnp.bfloat16),
            pltpu.VMEM((2 * HP, D), jnp.float32),
            pltpu.VMEM((D, 2 * HP), jnp.bfloat16),
            pltpu.VMEM((8, S), jnp.float32),
            pltpu.VMEM((2 * D + 16, S), jnp.bfloat16),
            pltpu.VMEM((S, 2 * HP), jnp.bfloat16),
            pltpu.VMEM((2 * HP, S), jnp.bfloat16),
            pltpu.VMEM((2 * HP, S), jnp.bfloat16),
            pltpu.VMEM((S, TQ), jnp.float32),
            pltpu.VMEM((S, TQ), jnp.float32),
            pltpu.VMEM((1, TQ), jnp.float32),
            pltpu.VMEM((1, TQ), jnp.float32),
        ],
        compiler_params=pltpu.CompilerParams(vmem_limit_bytes=100 * 1024 * 1024),
    )(xT, A_wqkv, A_wo, B_wqkv, B_wo, gate_w.reshape(1, D))
    return outT.T.reshape(1, S, D)
```

```python
import functools
import math

import jax
import jax.numpy as jnp
import jax.experimental.pallas as pl
import jax.experimental.pallas.tpu as pltpu

S, D, H, DH, DP = 2048, 448, 16, 28, 32
HP = H * DP
GW = 4 * DH
TQ = 1024
KC = 256
SUB = 256
NQ = S // TQ
NIT = 2 * H * NQ
NC = S // KC
NS = TQ // SUB
PC = 512
NP = S // PC
UN = 4
OC = 512
NO = S // OC


def _kernel(xT_hbm, wA_hbm, woA_hbm, wB_hbm, woB_hbm, gw_ref, o_hbm,
            xT_ref, w_ref, wo_ref, o_buf, sems,
            wT_scr, wopad_scr, woT_scr, g_scr, qT_scr, k_scr, vT_scr, oT_scr, sA, sB, mA, mB):
    f32, bf16 = jnp.float32, jnp.bfloat16

    def xcopy(c):
        c0 = pl.multiple_of(c * PC, PC)
        return pltpu.make_async_copy(xT_hbm.at[:, pl.ds(c0, PC)], xT_ref.at[:, pl.ds(c0, PC)], sems.at[4 + c])

    cps = [pltpu.make_async_copy(src, dst, sems.at[i]) for i, (src, dst) in enumerate(
        ((wA_hbm, w_ref.at[0]), (wB_hbm, w_ref.at[1]), (woA_hbm, wo_ref.at[0]), (woB_hbm, wo_ref.at[1])))]
    cps[0].start()
    for c in range(NP):
        xcopy(c).start()
    for cp in cps[1:]:
        cp.start()

    scale = (DH ** -0.5) * math.log2(math.e)
    r16 = jax.lax.broadcasted_iota(jnp.int32, (16, S), 0)
    slab = jnp.where(r16 == DH - 16, 1.0, 0.0).astype(bf16)
    def fill(i, carry):
        for t in range(4):
            vT_scr[pl.ds(pl.multiple_of((4 * i + t) * DP + 16, 16), 16), :] = slab
        for g in range(8):
            k_scr[pl.ds(pl.multiple_of(i * 256, 256), 256), g * 128 + GW:(g + 1) * 128] = jnp.zeros((256, 128 - GW), bf16)
        return carry
    jax.lax.fori_loop(0, 8, fill, 0)
    wopad_scr[...] = jnp.zeros_like(wopad_scr)
    qT_scr[2 * D:2 * D + 16, :] = jnp.zeros((16, S), bf16)
    gw8 = jnp.broadcast_to(gw_ref[...], (8, D))

    def step(it_qk, s_nxt, m_nxt, it_pv, s_cur, m_cur, extra=None):
        if it_qk is not None:
            h = it_qk // NQ
            qb = it_qk % NQ
            g = h // 4
            j = h % 4
            g0 = pl.multiple_of(g * 128, 128)
            gq0 = pl.multiple_of(g * GW, 16)
            q0 = pl.multiple_of(qb * TQ, TQ)
            qg = qT_scr[pl.ds(gq0, 128), pl.ds(q0, TQ)]
            rid = jax.lax.broadcasted_iota(jnp.int32, (128, 1), 0) - j * DH
            qm = jnp.where((rid >= 0) & (rid < DH), qg, jnp.zeros_like(qg))
        if it_pv is not None:
            h2 = it_pv // NQ
            qb2 = it_pv % NQ
            q02 = pl.multiple_of(qb2 * TQ, TQ)
            h02 = pl.multiple_of(h2 * DP, DP)
            mc = m_cur[...]
            gr = g_scr[pl.ds(h2 // H, 1), pl.ds(q02, TQ)]
        mx = [None] * NS
        o = [None] * NS
        for c in range(NC):
            if it_qk is not None:
                kg = k_scr[c * KC:(c + 1) * KC, pl.ds(g0, 128)]
            if it_pv is not None:
                vt = vT_scr[pl.ds(h02, DP), c * KC:(c + 1) * KC]
            for u in range(NS):
                cs = slice(u * SUB, (u + 1) * SUB)
                if it_qk is not None:
                    s = jnp.dot(kg, qm[:, cs], preferred_element_type=f32)
                    s_nxt[c * KC:(c + 1) * KC, cs] = s
                    sm = jnp.max(s.reshape(KC // 8, 8, SUB), axis=0)
                    mx[u] = sm if mx[u] is None else jnp.maximum(mx[u], sm)
                if extra is not None:
                    slot, nslot = c * NS + u, NC * NS
                    for t in range(len(extra)):
                        if (t * nslot) // len(extra) == slot:
                            extra[t]()
                if it_pv is not None:
                    p = jnp.exp2(s_cur[c * KC:(c + 1) * KC, cs] - mc[:, cs]).astype(bf16)
                    oc = jnp.dot(vt, p, preferred_element_type=f32)
                    o[u] = oc if o[u] is None else o[u] + oc
        for u in range(NS):
            cs = slice(u * SUB, (u + 1) * SUB)
            if it_qk is not None:
                m_nxt[:, cs] = jnp.max(mx[u], axis=0, keepdims=True)
            if it_pv is not None:
                qq = pl.multiple_of(q02 + u * SUB, SUB)
                r = gr[:, cs] / o[u][DH:DH + 1, :]
                oT_scr[pl.ds(h02, DP), pl.ds(qq, SUB)] = (o[u] * r).astype(bf16)

    def wo_pad(b):
        wo = wo_ref[b].astype(f32)
        for i in range(H):
            wopad_scr[b * HP + i * DP:b * HP + i * DP + DH, :] = wo[i * DH:(i + 1) * DH, :]

    def wo_xpose(k0):
        woT_scr[:, k0:k0 + 128] = wopad_scr[k0:k0 + 128, :].astype(bf16).T

    def wprep(blk, part):
        lo, hi = part
        wT_scr[lo:hi, :] = w_ref[blk, :, lo:hi].T

    wparts = [(0, 384), (384, 768), (768, 1152), (1152, 1344)]
    extra0 = ([functools.partial(wo_pad, b) for b in range(2)]
              + [functools.partial(wo_xpose, k0) for k0 in range(0, 2 * HP, 128)]
              + [functools.partial(wprep, 1, part) for part in wparts])

    def ocopy(c):
        c0 = pl.multiple_of(c * OC, OC)
        return pltpu.make_async_copy(o_buf.at[:, pl.ds(c0, OC)], o_hbm.at[:, pl.ds(c0, OC)], sems.at[4 + NP + c])

    def oproj_tile(n0):
        o_buf[:, n0:n0 + 128] = jnp.dot(woT_scr[...], oT_scr[:, n0:n0 + 128],
                                        preferred_element_type=f32).astype(bf16)

    oproj_early = [functools.partial(oproj_tile, n0) for n0 in range(0, S - TQ, 128)]

    def blk_body(blk, carry):
        b0 = pl.multiple_of(blk * HP, HP)
        bq0 = pl.multiple_of(blk * D, 16)

        def proj(c, carry):
            @pl.when(blk == 0)
            def _():
                xcopy(c).wait()
            c0 = pl.multiple_of(c * PC, PC)
            xTd = xT_ref[:, pl.ds(c0, PC)]
            qT = jnp.dot(wT_scr[0:D, :], xTd, preferred_element_type=f32)
            qT_scr[pl.ds(bq0, D), pl.ds(c0, PC)] = (qT * scale).astype(bf16)
            kT = jnp.dot(wT_scr[D:2 * D, :], xTd, preferred_element_type=f32).astype(bf16)
            for g in range(4):
                k_scr[pl.ds(c0, PC), pl.ds(pl.multiple_of(b0 + g * 128, 128), GW)] = kT[g * GW:(g + 1) * GW, :].T
            vT = jnp.dot(wT_scr[2 * D:3 * D, :], xTd, preferred_element_type=f32)
            for i in range(H):
                vT_scr[pl.ds(pl.multiple_of(b0 + i * DP, DP), DH), pl.ds(c0, PC)] = (
                    vT[i * DH:(i + 1) * DH, :].astype(bf16))
            gate = jax.nn.sigmoid(jnp.dot(gw8, xTd, preferred_element_type=f32)[0:1, :])
            g_scr[0:1, pl.ds(c0, PC)] = gate
            g_scr[1:2, pl.ds(c0, PC)] = 1.0 - gate
            return carry
        jax.lax.fori_loop(0, NP, proj, 0)

        @pl.when(blk == 0)
        def _():
            for cp in cps[1:]:
                cp.wait()
            step(0, sA, mA, None, None, None, extra=extra0)
        return carry

    cps[0].wait()
    for part in wparts:
        wprep(0, part)
    jax.lax.fori_loop(0, 2, blk_body, 0)

    def body(i, c):
        for u in range(UN // 2):
            it = UN * i + 2 * u
            step(it + 1, sB, mB, it, sA, mA)
            step(it + 2, sA, mA, it + 1, sB, mB)
        return c
    jax.lax.fori_loop(0, NIT // UN - 1, body, 0)
    for u in range(UN // 2):
        it = NIT - UN + 2 * u
        step(it + 1, sB, mB, it, sA, mA)
        if it + 2 < NIT:
            step(it + 2, sA, mA, it + 1, sB, mB)
        else:
            step(None, sA, mA, it + 1, sB, mB, extra=oproj_early)

    ne = (S - TQ) // OC
    for c in range(ne):
        ocopy(c).start()

    def oproj(c, carry):
        c0 = pl.multiple_of(c * OC, OC)
        o_buf[:, pl.ds(c0, OC)] = jnp.dot(woT_scr[...], oT_scr[:, pl.ds(c0, OC)],
                                          preferred_element_type=f32).astype(bf16)
        ocopy(c).start()
        return carry
    jax.lax.fori_loop(ne, NO, oproj, 0)
    for c in range(NO):
        ocopy(c).wait()


@jax.jit
def pallas_gated_mix__mha_block__mha_block__prompt_kernel(
    A_x: jax.Array,
    A_wqkv: jax.Array,
    A_wo: jax.Array,
    B_x: jax.Array,
    B_wqkv: jax.Array,
    B_wo: jax.Array,
    gate_w: jax.Array,
):
    del B_x
    xT = A_x.reshape(S, D).T
    any_spec = pl.BlockSpec(memory_space=pl.ANY)
    outT = pl.pallas_call(
        _kernel,
        out_shape=jax.ShapeDtypeStruct((D, S), jnp.bfloat16),
        in_specs=[any_spec] * 5 + [pl.BlockSpec(memory_space=pltpu.VMEM)],
        out_specs=any_spec,
        scratch_shapes=[
            pltpu.VMEM((D, S), jnp.bfloat16),
            pltpu.VMEM((2, D, 3 * D), jnp.bfloat16),
            pltpu.VMEM((2, D, D), jnp.bfloat16),
            pltpu.VMEM((D, S), jnp.bfloat16),
            pltpu.SemaphoreType.DMA((4 + NP + NO,)),
            pltpu.VMEM((3 * D, D), jnp.bfloat16),
            pltpu.VMEM((2 * HP, D), jnp.float32),
            pltpu.VMEM((D, 2 * HP), jnp.bfloat16),
            pltpu.VMEM((8, S), jnp.float32),
            pltpu.VMEM((2 * D + 16, S), jnp.bfloat16),
            pltpu.VMEM((S, 2 * HP), jnp.bfloat16),
            pltpu.VMEM((2 * HP, S), jnp.bfloat16),
            pltpu.VMEM((2 * HP, S), jnp.bfloat16),
            pltpu.VMEM((S, TQ), jnp.float32),
            pltpu.VMEM((S, TQ), jnp.float32),
            pltpu.VMEM((1, TQ), jnp.float32),
            pltpu.VMEM((1, TQ), jnp.float32),
        ],
        compiler_params=pltpu.CompilerParams(vmem_limit_bytes=100 * 1024 * 1024),
    )(xT, A_wqkv, A_wo, B_wqkv, B_wo, gate_w.reshape(1, D))
    return outT.T.reshape(1, S, D)
```

```python
import functools
import math

import jax
import jax.numpy as jnp
import jax.experimental.pallas as pl
import jax.experimental.pallas.tpu as pltpu

S, D, H, DH, DP = 2048, 448, 16, 28, 32
HP = H * DP
GW = 4 * DH
TQ = 1024
KC = 256
SUB = 256
NQ = S // TQ
NIT = 2 * H * NQ
NC = S // KC
NS = TQ // SUB
PC = 512
NP = S // PC
UN = 4
OC = 512
NO = S // OC


def _kernel(xT_hbm, wA_hbm, woA_hbm, wB_hbm, woB_hbm, gw_hbm, o_hbm,
            xT_ref, w_ref, wo_ref, gw_ref, o_buf, sems,
            wT_scr, wopad_scr, woT_scr, g_scr, qT_scr, k_scr, vT_scr, oT_scr, sA, sB, mA, mB):
    f32, bf16 = jnp.float32, jnp.bfloat16

    def xcopy(c):
        c0 = pl.multiple_of(c * PC, PC)
        return pltpu.make_async_copy(xT_hbm.at[:, pl.ds(c0, PC)], xT_ref.at[:, pl.ds(c0, PC)], sems.at[4 + c])

    cps = [pltpu.make_async_copy(src, dst, sems.at[i]) for i, (src, dst) in enumerate(
        ((wA_hbm, w_ref.at[0]), (wB_hbm, w_ref.at[1]), (woA_hbm, wo_ref.at[0]), (woB_hbm, wo_ref.at[1])))]
    gcp = pltpu.make_async_copy(gw_hbm, gw_ref, sems.at[4 + NP + NO])
    cps[0].start()
    gcp.start()
    for c in range(NP):
        xcopy(c).start()
    for cp in cps[1:]:
        cp.start()

    scale = (DH ** -0.5) * math.log2(math.e)
    r16 = jax.lax.broadcasted_iota(jnp.int32, (16, S), 0)
    slab = jnp.where(r16 == DH - 16, 1.0, 0.0).astype(bf16)
    def fill(i, carry):
        for t in range(4):
            vT_scr[pl.ds(pl.multiple_of((4 * i + t) * DP + 16, 16), 16), :] = slab
        for g in range(8):
            k_scr[pl.ds(pl.multiple_of(i * 256, 256), 256), g * 128 + GW:(g + 1) * 128] = jnp.zeros((256, 128 - GW), bf16)
        return carry
    jax.lax.fori_loop(0, 8, fill, 0)
    wopad_scr[...] = jnp.zeros_like(wopad_scr)
    qT_scr[2 * D:2 * D + 16, :] = jnp.zeros((16, S), bf16)

    def step(it_qk, s_nxt, m_nxt, it_pv, s_cur, m_cur, extra=None):
        if it_qk is not None:
            h = it_qk // NQ
            qb = it_qk % NQ
            g = h // 4
            j = h % 4
            g0 = pl.multiple_of(g * 128, 128)
            gq0 = pl.multiple_of(g * GW, 16)
            q0 = pl.multiple_of(qb * TQ, TQ)
            qg = qT_scr[pl.ds(gq0, 128), pl.ds(q0, TQ)]
            rid = jax.lax.broadcasted_iota(jnp.int32, (128, 1), 0) - j * DH
            qm = jnp.where((rid >= 0) & (rid < DH), qg, jnp.zeros_like(qg))
        if it_pv is not None:
            h2 = it_pv // NQ
            qb2 = it_pv % NQ
            q02 = pl.multiple_of(qb2 * TQ, TQ)
            h02 = pl.multiple_of(h2 * DP, DP)
            mc = m_cur[...]
            gr = g_scr[pl.ds(h2 // H, 1), pl.ds(q02, TQ)]
        mx = [None] * NS
        o = [None] * NS
        for c in range(NC):
            if it_qk is not None:
                kg = k_scr[c * KC:(c + 1) * KC, pl.ds(g0, 128)]
            if it_pv is not None:
                vt = vT_scr[pl.ds(h02, DP), c * KC:(c + 1) * KC]
            for u in range(NS):
                cs = slice(u * SUB, (u + 1) * SUB)
                if it_qk is not None:
                    s = jnp.dot(kg, qm[:, cs], preferred_element_type=f32)
                    s_nxt[c * KC:(c + 1) * KC, cs] = s
                    sm = jnp.max(s.reshape(KC // 8, 8, SUB), axis=0)
                    mx[u] = sm if mx[u] is None else jnp.maximum(mx[u], sm)
                if extra is not None:
                    slot, nslot = c * NS + u, NC * NS
                    for t in range(len(extra)):
                        if (t * nslot) // len(extra) == slot:
                            extra[t]()
                if it_pv is not None:
                    p = jnp.exp2(s_cur[c * KC:(c + 1) * KC, cs] - mc[:, cs]).astype(bf16)
                    oc = jnp.dot(vt, p, preferred_element_type=f32)
                    o[u] = oc if o[u] is None else o[u] + oc
        for u in range(NS):
            cs = slice(u * SUB, (u + 1) * SUB)
            if it_qk is not None:
                m_nxt[:, cs] = jnp.max(mx[u], axis=0, keepdims=True)
            if it_pv is not None:
                qq = pl.multiple_of(q02 + u * SUB, SUB)
                r = gr[:, cs] / o[u][DH:DH + 1, :]
                oT_scr[pl.ds(h02, DP), pl.ds(qq, SUB)] = (o[u] * r).astype(bf16)

    def wo_pad(b):
        wo = wo_ref[b].astype(f32)
        for i in range(H):
            wopad_scr[b * HP + i * DP:b * HP + i * DP + DH, :] = wo[i * DH:(i + 1) * DH, :]

    def wo_xpose(k0):
        woT_scr[:, k0:k0 + 128] = wopad_scr[k0:k0 + 128, :].astype(bf16).T

    def wprep(blk, part):
        lo, hi = part
        wT_scr[lo:hi, :] = w_ref[blk, :, lo:hi].T

    wparts = [(0, 384), (384, 768), (768, 1152), (1152, 1344)]
    extra0 = ([functools.partial(wo_pad, b) for b in range(2)]
              + [functools.partial(wo_xpose, k0) for k0 in range(0, 2 * HP, 128)]
              + [functools.partial(wprep, 1, part) for part in wparts])

    def ocopy(c):
        c0 = pl.multiple_of(c * OC, OC)
        return pltpu.make_async_copy(o_buf.at[:, pl.ds(c0, OC)], o_hbm.at[:, pl.ds(c0, OC)], sems.at[4 + NP + c])

    def oproj_tile(n0):
        o_buf[:, n0:n0 + 128] = jnp.dot(woT_scr[...], oT_scr[:, n0:n0 + 128],
                                        preferred_element_type=f32).astype(bf16)

    oproj_early = [functools.partial(oproj_tile, n0) for n0 in range(0, S - TQ, 128)]

    def blk_body(blk, carry):
        b0 = pl.multiple_of(blk * HP, HP)
        bq0 = pl.multiple_of(blk * D, 16)

        def proj(c, carry):
            @pl.when(blk == 0)
            def _():
                xcopy(c).wait()
            c0 = pl.multiple_of(c * PC, PC)
            xTd = xT_ref[:, pl.ds(c0, PC)]
            qT = jnp.dot(wT_scr[0:D, :], xTd, preferred_element_type=f32)
            qT_scr[pl.ds(bq0, D), pl.ds(c0, PC)] = (qT * scale).astype(bf16)
            kT = jnp.dot(wT_scr[D:2 * D, :], xTd, preferred_element_type=f32).astype(bf16)
            for g in range(4):
                k_scr[pl.ds(c0, PC), pl.ds(pl.multiple_of(b0 + g * 128, 128), GW)] = kT[g * GW:(g + 1) * GW, :].T
            vT = jnp.dot(wT_scr[2 * D:3 * D, :], xTd, preferred_element_type=f32)
            for i in range(H):
                vT_scr[pl.ds(pl.multiple_of(b0 + i * DP, DP), DH), pl.ds(c0, PC)] = (
                    vT[i * DH:(i + 1) * DH, :].astype(bf16))
            gate = jax.nn.sigmoid(jnp.dot(gw8, xTd, preferred_element_type=f32)[0:1, :])
            g_scr[0:1, pl.ds(c0, PC)] = gate
            g_scr[1:2, pl.ds(c0, PC)] = 1.0 - gate
            return carry
        jax.lax.fori_loop(0, NP, proj, 0)

        @pl.when(blk == 0)
        def _():
            for cp in cps[1:]:
                cp.wait()
            step(0, sA, mA, None, None, None, extra=extra0)
        return carry

    cps[0].wait()
    gcp.wait()
    gw8 = jnp.broadcast_to(gw_ref[...].reshape(1, D), (8, D))
    for part in wparts:
        wprep(0, part)
    jax.lax.fori_loop(0, 2, blk_body, 0)

    def body(i, c):
        for u in range(UN // 2):
            it = UN * i + 2 * u
            step(it + 1, sB, mB, it, sA, mA)
            step(it + 2, sA, mA, it + 1, sB, mB)
        return c
    jax.lax.fori_loop(0, NIT // UN - 1, body, 0)
    for u in range(UN // 2):
        it = NIT - UN + 2 * u
        step(it + 1, sB, mB, it, sA, mA)
        if it + 2 < NIT:
            step(it + 2, sA, mA, it + 1, sB, mB)
        else:
            step(None, sA, mA, it + 1, sB, mB, extra=oproj_early)

    ne = (S - TQ) // OC
    for c in range(ne):
        ocopy(c).start()

    def oproj(c, carry):
        c0 = pl.multiple_of(c * OC, OC)
        o_buf[:, pl.ds(c0, OC)] = jnp.dot(woT_scr[...], oT_scr[:, pl.ds(c0, OC)],
                                          preferred_element_type=f32).astype(bf16)
        ocopy(c).start()
        return carry
    jax.lax.fori_loop(ne, NO, oproj, 0)
    for c in range(NO):
        ocopy(c).wait()


@jax.jit
def pallas_gated_mix__mha_block__mha_block__prompt_kernel(
    A_x: jax.Array,
    A_wqkv: jax.Array,
    A_wo: jax.Array,
    B_x: jax.Array,
    B_wqkv: jax.Array,
    B_wo: jax.Array,
    gate_w: jax.Array,
):
    del B_x
    xT = A_x.reshape(S, D).T
    any_spec = pl.BlockSpec(memory_space=pl.ANY)
    outT = pl.pallas_call(
        _kernel,
        out_shape=jax.ShapeDtypeStruct((D, S), jnp.bfloat16),
        in_specs=[any_spec] * 6,
        out_specs=any_spec,
        scratch_shapes=[
            pltpu.VMEM((D, S), jnp.bfloat16),
            pltpu.VMEM((2, D, 3 * D), jnp.bfloat16),
            pltpu.VMEM((2, D, D), jnp.bfloat16),
            pltpu.VMEM((D,), jnp.bfloat16),
            pltpu.VMEM((D, S), jnp.bfloat16),
            pltpu.SemaphoreType.DMA((4 + NP + NO + 1,)),
            pltpu.VMEM((3 * D, D), jnp.bfloat16),
            pltpu.VMEM((2 * HP, D), jnp.float32),
            pltpu.VMEM((D, 2 * HP), jnp.bfloat16),
            pltpu.VMEM((8, S), jnp.float32),
            pltpu.VMEM((2 * D + 16, S), jnp.bfloat16),
            pltpu.VMEM((S, 2 * HP), jnp.bfloat16),
            pltpu.VMEM((2 * HP, S), jnp.bfloat16),
            pltpu.VMEM((2 * HP, S), jnp.bfloat16),
            pltpu.VMEM((S, TQ), jnp.float32),
            pltpu.VMEM((S, TQ), jnp.float32),
            pltpu.VMEM((1, TQ), jnp.float32),
            pltpu.VMEM((1, TQ), jnp.float32),
        ],
        compiler_params=pltpu.CompilerParams(vmem_limit_bytes=100 * 1024 * 1024),
    )(xT, A_wqkv, A_wo, B_wqkv, B_wo, gate_w)
    return outT.T.reshape(1, S, D)
```
